```python
import os as _os
_os.environ.setdefault("JAX_PLATFORMS", "cpu")
import jax
import jax.numpy as jnp

def _softmax(x, axis=-1):
    return jax.nn.softmax(x, axis=axis)
def _gelu(x):
    return jax.nn.gelu(x, approximate=True)
def _silu(x):
    return jax.nn.silu(x)
def _sigmoid(x):
    return jax.nn.sigmoid(x)
def _layernorm(x, axis=-1, eps=1e-5):
    m = jnp.mean(x, axis=axis, keepdims=True)
    v = jnp.var(x, axis=axis, keepdims=True)
    return (x - m) / jnp.sqrt(v + eps)
def _scatter_add(tgt, idx, src, axis=0):
    return tgt.at[idx].add(src)
def _segment_sum(src, seg, n):
    return jax.ops.segment_sum(src, seg, n)
class _Rng:
    def __init__(self, key):
        self._k = key
    def _next(self):
        self._k, sub = jax.random.split(self._k)
        return sub
    def normal(self, shape):
        return jax.random.normal(self._next(), shape, dtype=jnp.bfloat16)
    def randint(self, lo, hi, shape):
        return jax.random.randint(self._next(), shape, lo, hi, dtype=jnp.int32)
    def uniform(self, shape, lo=0.0, hi=1.0):
        return jax.random.uniform(self._next(), shape, jnp.bfloat16, lo, hi)
    def permutation(self, n):
        return jax.random.permutation(self._next(), n)


kernel_name = 'sequential_preLN__spectral_gfnet__glu_gated_bilinear__prompt'

def setup_inputs():
    _rng = _Rng(jax.random.key(int.from_bytes(__import__("os").urandom(4), "little")))
    _w = (lambda a: (lambda t: t.astype(jnp.bfloat16) if jnp.issubdtype(t.dtype, jnp.floating) else t)(jnp.asarray(a)))
    def _A_setup():
        B, S, D = 1, 2048, 448
        Df = D // 2 + 1
        return {
            "x": _w((lambda *s: _rng.normal(s) * 0.05)(B, S, D)),
            "w_r": _w((lambda *s: _rng.normal(s) * 0.2)(S, Df) * 0.02),
            "w_i": _w((lambda *s: _rng.normal(s) * 0.2)(S, Df) * 0.02),
        }
    _A_in = _A_setup()

    def _B_setup():
        B, S, D, F = 1, 2048, 448, 1792
        return {
            "x": _w((lambda *s: _rng.normal(s) * 0.05)(B, S, D)),
            "w_gate": _w((lambda *s: _rng.normal(s) * 0.05)(D, F) * (D ** -0.5)),
            "w_up": _w((lambda *s: _rng.normal(s) * 0.05)(D, F) * (D ** -0.5)),
            "w_down": _w((lambda *s: _rng.normal(s) * 0.05)(F, D) * (F ** -0.5)),
        }
    _B_in = _B_setup()

    return {
        "A_x": _A_in["x"],
        "A_w_r": _A_in["w_r"],
        "A_w_i": _A_in["w_i"],
        "B_x": _B_in["x"],
        "B_w_gate": _B_in["w_gate"],
        "B_w_up": _B_in["w_up"],
        "B_w_down": _B_in["w_down"],
    }

def reference(A_x, A_w_r, A_w_i, B_x, B_w_gate, B_w_up, B_w_down):
    def _A_ref(x, w_r, w_i):
        B, S, D = x.shape
        X = (lambda x, axes=(-2,-1): jnp.fft.rfft2(x.astype(jnp.float32), axes=axes))(x, axes=(-2, -1))
        W = w_r + 1j * w_i
        X = X * W
        y = (lambda x, s, axes=(-2,-1): jnp.fft.irfft2(x, s=s, axes=axes).astype(jnp.bfloat16))(X, (S, D), axes=(-2, -1))
        return y

    def _B_ref(x, w_gate, w_up, w_down):
        g = jnp.einsum("bsd,df->bsf", x, w_gate)
        u = jnp.einsum("bsd,df->bsf", x, w_up)
        h = g * u
        return jnp.einsum("bsf,fd->bsd", h, w_down)

    x = A_x
    h = x + _A_ref(_layernorm(x, axis=-1), A_w_r, A_w_i)
    h2 = h + _B_ref(_layernorm(h, axis=-1), B_w_gate, B_w_up, B_w_down)
    return h2
```

```python
import functools

import numpy as np
import jax
import jax.numpy as jnp
import jax.experimental.pallas as pl
import jax.experimental.pallas.tpu as pltpu

S = 2048
D = 448
DF = D // 2 + 1
F = 1792
NS = 16
R = 128
PW = 256
EPS = 1e-5
BM = 512
FC = 256
CH = 256


def _dft_constants():
    d = np.arange(D)[:, None]
    f = np.arange(DF)[None, :]
    ang = 2.0 * np.pi * ((d * f) % D) / D
    fd = np.zeros((D, 2 * PW), np.float64)
    fd[:, :DF] = np.cos(ang)
    fd[:, PW:PW + DF] = -np.sin(ang)
    c = np.full((DF,), 2.0)
    c[0] = 1.0
    c[DF - 1] = 1.0
    gd = np.zeros((2 * PW, D), np.float64)
    gd[:DF] = c[:, None] * np.cos(ang.T) / (D * S)
    gd[PW:PW + DF] = -c[:, None] * np.sin(ang.T) / (D * S)
    n2 = np.arange(R)
    k2 = np.arange(R)
    mf = np.zeros((NS, 2 * R, R), np.float64)
    mi = np.zeros((NS, 2 * R, R), np.float64)
    for k1 in range(NS):
        a = 2.0 * np.pi * (((k1 + NS * k2)[:, None] * n2[None, :]) % S) / S
        mf[k1, :R] = np.cos(a)
        mf[k1, R:] = -np.sin(a)
        mi[k1, :R] = np.cos(a.T)
        mi[k1, R:] = np.sin(a.T)
    bf = jnp.bfloat16
    return (jnp.asarray(fd, bf), jnp.asarray(gd, bf),
            jnp.asarray(mf.reshape(NS * 2 * R, R), bf),
            jnp.asarray(mi.reshape(NS * 2 * R, R), bf))


def _radix4(a0, a1, a2, a3, sign):
    t0 = (a0[0] + a2[0], a0[1] + a2[1])
    t1 = (a0[0] - a2[0], a0[1] - a2[1])
    t2 = (a1[0] + a3[0], a1[1] + a3[1])
    t3 = (a1[0] - a3[0], a1[1] - a3[1])
    y0 = (t0[0] + t2[0], t0[1] + t2[1])
    y2 = (t0[0] - t2[0], t0[1] - t2[1])
    if sign < 0:
        y1 = (t1[0] + t3[1], t1[1] - t3[0])
        y3 = (t1[0] - t3[1], t1[1] + t3[0])
    else:
        y1 = (t1[0] - t3[1], t1[1] + t3[0])
        y3 = (t1[0] + t3[1], t1[1] - t3[0])
    return y0, y1, y2, y3


def _cmul_const(a, e, sign):
    e = e % 16
    if e == 0:
        return a
    th = sign * 2.0 * np.pi * e / 16.0
    cr = float(np.cos(th))
    ci = float(np.sin(th))
    if e == 4 or e == 12:
        ci = float(np.round(ci))
        return (-ci * a[1], ci * a[0]) if ci > 0 else (a[1], -a[0])
    if e == 8:
        return (-a[0], -a[1])
    return (a[0] * cr - a[1] * ci, a[0] * ci + a[1] * cr)


def _radix16(a, sign):
    b = [None] * 4
    for q in range(4):
        b[q] = _radix4(a[q], a[4 + q], a[8 + q], a[12 + q], sign)
    out = [None] * 16
    for r in range(4):
        c = [_cmul_const(b[q][r], q * r, sign) for q in range(4)]
        y = _radix4(c[0], c[1], c[2], c[3], sign)
        for t in range(4):
            out[r + 4 * t] = y[t]
    return out


def _layernorm(v):
    m = jnp.mean(v, axis=-1, keepdims=True)
    c = v - m
    var = jnp.mean(c * c, axis=-1, keepdims=True)
    return c * jax.lax.rsqrt(var + EPS)


def _kernel(x_ref, fd_ref, wr_ref, wi_ref, mf_hbm, mi_hbm, gd_hbm, wg_hbm, wu_hbm, wd_hbm,
            o_ref,
            xs, h_scr, wf, mf_v, mi_v, gd_v, wg_v, wu_v, wd_v, sems):
    step = pl.program_id(0)
    f32 = jnp.float32
    bf16 = jnp.bfloat16

    def _copies():
        pairs = [(mf_hbm, mf_v), (mi_hbm, mi_v), (gd_hbm, gd_v),
                 (wg_hbm, wg_v), (wu_hbm, wu_v), (wd_hbm, wd_v)]
        return [pltpu.make_async_copy(s, d, sems.at[j]) for j, (s, d) in enumerate(pairs)]

    def _slab_butterflies(sign):
        def body(c, carry):
            r0 = pl.multiple_of((c // 2) * 8, 8)
            l0 = (c % 2) * 128
            for lane in (0, 128):
                @pl.when(l0 == lane)
                def _():
                    a = []
                    for n in range(NS):
                        rows = pl.ds(n * R + r0, 8)
                        a.append((xs[rows, lane:lane + 128], xs[rows, PW + lane:PW + lane + 128]))
                    y = _radix16(a, sign)
                    for n in range(NS):
                        rows = pl.ds(n * R + r0, 8)
                        xs[rows, lane:lane + 128] = y[n][0]
                        xs[rows, PW + lane:PW + lane + 128] = y[n][1]
            return carry
        jax.lax.fori_loop(0, (R // 8) * 2, body, 0)

    @pl.when(step == 0)
    def _spectral():
        cps = _copies()
        for cp in cps:
            cp.start()

        for c in range(S // CH):
            rows = pl.ds(c * CH, CH)
            for j, w_ref in enumerate((wr_ref, wi_ref)):
                wf[2 * j, rows, :] = w_ref[rows, :128].astype(f32)
                wf[2 * j + 1, rows, :] = jnp.zeros((CH, 128), f32)
                wf[2 * j + 1, rows, :DF - 128] = w_ref[rows, 128:].astype(f32)

        for c in range(S // CH):
            rows = pl.ds(c * CH, CH)
            xn = _layernorm(x_ref[rows, :].astype(f32)).astype(bf16)
            xs[rows, :] = jnp.dot(xn, fd_ref[...], preferred_element_type=f32)

        _slab_butterflies(-1)

        cps[0].wait()
        cps[1].wait()
        for k1 in range(NS):
            rows = pl.ds(k1 * R, R)
            y = xs[rows, :].astype(bf16)
            p = jnp.dot(mf_v[pl.ds(k1 * 2 * R, 2 * R), :], y, preferred_element_type=f32)
            zr = p[:R, :PW] - p[R:, PW:]
            zi = p[R:, :PW] + p[:R, PW:]
            fr = jnp.concatenate([wf[0, pl.ds(k1, R, stride=NS), :],
                                  wf[1, pl.ds(k1, R, stride=NS), :]], axis=1)
            fi = jnp.concatenate([wf[2, pl.ds(k1, R, stride=NS), :],
                                  wf[3, pl.ds(k1, R, stride=NS), :]], axis=1)
            z = jnp.concatenate([zr * fr - zi * fi, zr * fi + zi * fr], axis=1).astype(bf16)
            q = jnp.dot(mi_v[pl.ds(k1 * 2 * R, 2 * R), :], z, preferred_element_type=f32)
            xs[rows, :] = jnp.concatenate(
                [q[:R, :PW] - q[R:, PW:], q[R:, :PW] + q[:R, PW:]], axis=1)

        _slab_butterflies(+1)

        cps[2].wait()
        for c in range(S // CH):
            rows = pl.ds(c * CH, CH)
            y = jnp.dot(xs[rows, :].astype(bf16), gd_v[...], preferred_element_type=f32)
            h_scr[rows, :] = x_ref[rows, :] + y.astype(bf16)

        cps[3].wait()
        cps[4].wait()
        cps[5].wait()

    rows = pl.ds(pl.multiple_of(step * BM, BM), BM)
    h = h_scr[rows, :]
    ln = _layernorm(h.astype(f32)).astype(bf16)
    acc = jnp.zeros((BM, D), f32)
    for c in range(F // FC):
        g = jnp.dot(ln, wg_v[:, c * FC:(c + 1) * FC], preferred_element_type=f32)
        u = jnp.dot(ln, wu_v[:, c * FC:(c + 1) * FC], preferred_element_type=f32)
        a = (g * u).astype(bf16)
        acc = acc + jnp.dot(a, wd_v[c * FC:(c + 1) * FC, :], preferred_element_type=f32)
    o_ref[...] = h + acc.astype(bf16)


@jax.jit
def pallas_sequential_preLN__spectral_gfnet__glu_gated_bilinear__prompt_kernel(
    A_x: jax.Array,
    A_w_r: jax.Array,
    A_w_i: jax.Array,
    B_x: jax.Array,
    B_w_gate: jax.Array,
    B_w_up: jax.Array,
    B_w_down: jax.Array,
):
    del B_x
    x = A_x.reshape(S, D)
    fd, gd, mf, mi = _dft_constants()
    full = lambda shape: pl.BlockSpec(shape, lambda i: (0,) * len(shape))
    hbm = pl.BlockSpec(memory_space=pl.ANY)
    out = pl.pallas_call(
        _kernel,
        grid=(S // BM,),
        in_specs=[full((S, D)), full((D, 2 * PW)), full((S, DF)), full((S, DF)),
                  hbm, hbm, hbm, hbm, hbm, hbm],
        out_specs=pl.BlockSpec((BM, D), lambda i: (i, 0)),
        out_shape=jax.ShapeDtypeStruct((S, D), jnp.bfloat16),
        scratch_shapes=[
            pltpu.VMEM((S, 2 * PW), jnp.float32),
            pltpu.VMEM((S, D), jnp.bfloat16),
            pltpu.VMEM((4, S, 128), jnp.float32),
            pltpu.VMEM((NS * 2 * R, R), jnp.bfloat16),
            pltpu.VMEM((NS * 2 * R, R), jnp.bfloat16),
            pltpu.VMEM((2 * PW, D), jnp.bfloat16),
            pltpu.VMEM((D, F), jnp.bfloat16),
            pltpu.VMEM((D, F), jnp.bfloat16),
            pltpu.VMEM((F, D), jnp.bfloat16),
            pltpu.SemaphoreType.DMA((6,)),
        ],
        compiler_params=pltpu.CompilerParams(
            dimension_semantics=("arbitrary",),
            vmem_limit_bytes=100 * 1024 * 1024,
        ),
    )(x, fd, A_w_r, A_w_i, mf, mi, gd, B_w_gate, B_w_up, B_w_down)
    return out.reshape(1, S, D)
```

```python
import numpy as np
import jax
import jax.numpy as jnp
import jax.experimental.pallas as pl
import jax.experimental.pallas.tpu as pltpu

S = 2048
D = 448
DF = D // 2 + 1
F = 1792
NS = 16
R = 128
PW = 256
EPS = 1e-5
BN = 512
FC = 256
CN = 512


def _dft_constants():
    d = np.arange(D)[None, :]
    f = np.arange(DF)[:, None]
    ang = 2.0 * np.pi * ((d * f) % D) / D
    fdt = np.zeros((2 * PW, D), np.float64)
    fdt[:DF] = np.cos(ang)
    fdt[PW:PW + DF] = -np.sin(ang)
    c = np.full((DF,), 2.0)
    c[0] = 1.0
    c[DF - 1] = 1.0
    gdt = np.zeros((D, 2 * PW), np.float64)
    gdt[:, :DF] = (c[:, None] * np.cos(ang)).T / (D * S)
    gdt[:, PW:PW + DF] = -(c[:, None] * np.sin(ang)).T / (D * S)
    n2 = np.arange(R)
    k2 = np.arange(R)
    mf = np.zeros((NS, R, 2 * R), np.float64)
    mi = np.zeros((NS, R, 2 * R), np.float64)
    for k1 in range(NS):
        a = 2.0 * np.pi * ((n2[:, None] * (k1 + NS * k2)[None, :]) % S) / S
        mf[k1, :, :R] = np.cos(a)
        mf[k1, :, R:] = -np.sin(a)
        mi[k1, :, :R] = np.cos(a.T)
        mi[k1, :, R:] = np.sin(a.T)
    bf = jnp.bfloat16
    return (jnp.asarray(fdt, bf), jnp.asarray(gdt, bf),
            jnp.asarray(mf.reshape(NS * R, 2 * R), bf),
            jnp.asarray(mi.reshape(NS * R, 2 * R), bf))


def _radix4(a0, a1, a2, a3, sign):
    t0 = (a0[0] + a2[0], a0[1] + a2[1])
    t1 = (a0[0] - a2[0], a0[1] - a2[1])
    t2 = (a1[0] + a3[0], a1[1] + a3[1])
    t3 = (a1[0] - a3[0], a1[1] - a3[1])
    y0 = (t0[0] + t2[0], t0[1] + t2[1])
    y2 = (t0[0] - t2[0], t0[1] - t2[1])
    if sign < 0:
        y1 = (t1[0] + t3[1], t1[1] - t3[0])
        y3 = (t1[0] - t3[1], t1[1] + t3[0])
    else:
        y1 = (t1[0] - t3[1], t1[1] + t3[0])
        y3 = (t1[0] + t3[1], t1[1] - t3[0])
    return y0, y1, y2, y3


def _cmul_const(a, e, sign):
    e = e % 16
    if e == 0:
        return a
    if e == 8:
        return (-a[0], -a[1])
    if e == 4 or e == 12:
        plus_i = (sign > 0) == (e == 4)
        return (-a[1], a[0]) if plus_i else (a[1], -a[0])
    th = sign * 2.0 * np.pi * e / 16.0
    cr = float(np.cos(th))
    ci = float(np.sin(th))
    return (a[0] * cr - a[1] * ci, a[0] * ci + a[1] * cr)


def _radix16(a, sign):
    b = [None] * 4
    for q in range(4):
        b[q] = _radix4(a[q], a[4 + q], a[8 + q], a[12 + q], sign)
    out = [None] * 16
    for r in range(4):
        c = [_cmul_const(b[q][r], q * r, sign) for q in range(4)]
        y = _radix4(c[0], c[1], c[2], c[3], sign)
        for t in range(4):
            out[r + 4 * t] = y[t]
    return out


def _layernorm0(v):
    m = jnp.mean(v, axis=0, keepdims=True)
    c = v - m
    var = jnp.mean(c * c, axis=0, keepdims=True)
    return c * jax.lax.rsqrt(var + EPS)


def _kernel(x_ref, fdt_ref, wr_ref, wi_ref, mf_hbm, mi_hbm, gdt_hbm, wg_hbm, wu_hbm, wdt_hbm,
            o_ref,
            xs, h_scr, mf_v, mi_v, gdt_v, wg_v, wu_v, wdt_v, wgt, wut, sems):
    step = pl.program_id(0)
    f32 = jnp.float32
    bf16 = jnp.bfloat16

    def _copies():
        pairs = [(mf_hbm, mf_v), (mi_hbm, mi_v), (gdt_hbm, gdt_v),
                 (wg_hbm, wg_v), (wu_hbm, wu_v), (wdt_hbm, wdt_v)]
        return [pltpu.make_async_copy(s, d, sems.at[j]) for j, (s, d) in enumerate(pairs)]

    def _tile_butterflies(sign):
        def body(c, carry):
            r0 = pl.multiple_of(c * 8, 8)
            a = []
            for n in range(NS):
                a.append((xs[pl.ds(r0, 8), n * R:(n + 1) * R],
                          xs[pl.ds(PW + r0, 8), n * R:(n + 1) * R]))
            y = _radix16(a, sign)
            for n in range(NS):
                xs[pl.ds(r0, 8), n * R:(n + 1) * R] = y[n][0]
                xs[pl.ds(PW + r0, 8), n * R:(n + 1) * R] = y[n][1]
            return carry
        jax.lax.fori_loop(0, PW // 8, body, 0)

    @pl.when(step == 0)
    def _spectral():
        cps = _copies()
        for cp in cps:
            cp.start()

        for c in range(S // CN):
            cols = slice(c * CN, (c + 1) * CN)
            xn = _layernorm0(x_ref[:, cols].astype(f32)).astype(bf16)
            xs[:, cols] = jnp.dot(fdt_ref[...], xn, preferred_element_type=f32)

        _tile_butterflies(-1)

        cps[0].wait()
        cps[1].wait()
        for k1 in range(NS):
            cols = slice(k1 * R, (k1 + 1) * R)
            y = xs[:, cols].astype(bf16)
            p = jnp.dot(y, mf_v[pl.ds(k1 * R, R), :], preferred_element_type=f32)
            zr = p[:PW, :R] - p[PW:, R:]
            zi = p[:PW, R:] + p[PW:, :R]
            fr = wr_ref[:, cols].astype(f32)
            fi = wi_ref[:, cols].astype(f32)
            z = jnp.concatenate([zr * fr - zi * fi, zr * fi + zi * fr], axis=0).astype(bf16)
            q = jnp.dot(z, mi_v[pl.ds(k1 * R, R), :], preferred_element_type=f32)
            xs[:, cols] = jnp.concatenate(
                [q[:PW, :R] - q[PW:, R:], q[:PW, R:] + q[PW:, :R]], axis=0)

        _tile_butterflies(+1)

        cps[2].wait()
        for c in range(S // CN):
            cols = slice(c * CN, (c + 1) * CN)
            y = jnp.dot(gdt_v[...], xs[:, cols].astype(bf16), preferred_element_type=f32)
            h_scr[:, cols] = x_ref[:, cols] + y.astype(bf16)

        cps[3].wait()
        cps[4].wait()
        cps[5].wait()
        for c in range(F // FC):
            wgt[c * FC:(c + 1) * FC, :] = wg_v[:, c * FC:(c + 1) * FC].T
            wut[c * FC:(c + 1) * FC, :] = wu_v[:, c * FC:(c + 1) * FC].T

    cols = pl.ds(pl.multiple_of(step * BN, BN), BN)
    h = h_scr[:, cols]
    ln = _layernorm0(h.astype(f32)).astype(bf16)
    acc = jnp.zeros((D, BN), f32)
    for c in range(F // FC):
        g = jnp.dot(wgt[c * FC:(c + 1) * FC, :], ln, preferred_element_type=f32)
        u = jnp.dot(wut[c * FC:(c + 1) * FC, :], ln, preferred_element_type=f32)
        a = (g * u).astype(bf16)
        acc = acc + jnp.dot(wdt_v[:, c * FC:(c + 1) * FC], a, preferred_element_type=f32)
    o_ref[...] = h + acc.astype(bf16)


def _digit_reversed_filter(w):
    wt = jnp.pad(w.T, ((0, PW - DF), (0, 0)))
    return wt.reshape(PW, R, NS).swapaxes(1, 2).reshape(PW, S)


@jax.jit
def pallas_sequential_preLN__spectral_gfnet__glu_gated_bilinear__prompt_kernel(
    A_x: jax.Array,
    A_w_r: jax.Array,
    A_w_i: jax.Array,
    B_x: jax.Array,
    B_w_gate: jax.Array,
    B_w_up: jax.Array,
    B_w_down: jax.Array,
):
    del B_x
    xt = A_x.reshape(S, D).T
    fdt, gdt, mf, mi = _dft_constants()
    full = lambda shape: pl.BlockSpec(shape, lambda i: (0,) * len(shape))
    hbm = pl.BlockSpec(memory_space=pl.ANY)
    out = pl.pallas_call(
        _kernel,
        grid=(S // BN,),
        in_specs=[full((D, S)), full((2 * PW, D)), full((PW, S)), full((PW, S)),
                  hbm, hbm, hbm, hbm, hbm, hbm],
        out_specs=pl.BlockSpec((D, BN), lambda i: (0, i)),
        out_shape=jax.ShapeDtypeStruct((D, S), jnp.bfloat16),
        scratch_shapes=[
            pltpu.VMEM((2 * PW, S), jnp.float32),
            pltpu.VMEM((D, S), jnp.bfloat16),
            pltpu.VMEM((NS * R, 2 * R), jnp.bfloat16),
            pltpu.VMEM((NS * R, 2 * R), jnp.bfloat16),
            pltpu.VMEM((D, 2 * PW), jnp.bfloat16),
            pltpu.VMEM((D, F), jnp.bfloat16),
            pltpu.VMEM((D, F), jnp.bfloat16),
            pltpu.VMEM((D, F), jnp.bfloat16),
            pltpu.VMEM((F, D), jnp.bfloat16),
            pltpu.VMEM((F, D), jnp.bfloat16),
            pltpu.SemaphoreType.DMA((6,)),
        ],
        compiler_params=pltpu.CompilerParams(
            dimension_semantics=("arbitrary",),
            vmem_limit_bytes=100 * 1024 * 1024,
        ),
    )(xt, fdt, _digit_reversed_filter(A_w_r), _digit_reversed_filter(A_w_i),
      mf, mi, gdt, B_w_gate, B_w_up, B_w_down.T)
    return out.T.reshape(1, S, D)
```

```python
import numpy as np
import jax
import jax.numpy as jnp
import jax.experimental.pallas as pl
import jax.experimental.pallas.tpu as pltpu

S = 2048
D = 448
DF = D // 2 + 1
F = 1792
NS = 16
R = 128
PW = 256
EPS = 1e-5
BN = 512
FC = 256
CN = 512


def _dft_constants():
    d = np.arange(D)[None, :]
    f = np.arange(DF)[:, None]
    ang = 2.0 * np.pi * ((d * f) % D) / D
    fdt = np.zeros((2 * PW, D), np.float64)
    fdt[:DF] = np.cos(ang)
    fdt[PW:PW + DF] = -np.sin(ang)
    c = np.full((DF,), 2.0)
    c[0] = 1.0
    c[DF - 1] = 1.0
    gdt = np.zeros((D, 2 * PW), np.float64)
    gdt[:, :DF] = (c[:, None] * np.cos(ang)).T / (D * S)
    gdt[:, PW:PW + DF] = -(c[:, None] * np.sin(ang)).T / (D * S)
    n2 = np.arange(R)
    k2 = np.arange(R)
    mf = np.zeros((NS, R, 2 * R), np.float64)
    mi = np.zeros((NS, R, 2 * R), np.float64)
    for k1 in range(NS):
        a = 2.0 * np.pi * ((n2[:, None] * (k1 + NS * k2)[None, :]) % S) / S
        mf[k1, :, :R] = np.cos(a)
        mf[k1, :, R:] = -np.sin(a)
        mi[k1, :, :R] = np.cos(a.T)
        mi[k1, :, R:] = np.sin(a.T)
    bf = jnp.bfloat16
    return (jnp.asarray(fdt, bf), jnp.asarray(gdt, bf),
            jnp.asarray(mf.reshape(NS * R, 2 * R), bf),
            jnp.asarray(mi.reshape(NS * R, 2 * R), bf))


def _radix4(a0, a1, a2, a3, sign):
    t0 = (a0[0] + a2[0], a0[1] + a2[1])
    t1 = (a0[0] - a2[0], a0[1] - a2[1])
    t2 = (a1[0] + a3[0], a1[1] + a3[1])
    t3 = (a1[0] - a3[0], a1[1] - a3[1])
    y0 = (t0[0] + t2[0], t0[1] + t2[1])
    y2 = (t0[0] - t2[0], t0[1] - t2[1])
    if sign < 0:
        y1 = (t1[0] + t3[1], t1[1] - t3[0])
        y3 = (t1[0] - t3[1], t1[1] + t3[0])
    else:
        y1 = (t1[0] - t3[1], t1[1] + t3[0])
        y3 = (t1[0] + t3[1], t1[1] - t3[0])
    return y0, y1, y2, y3


def _cmul_const(a, e, sign):
    e = e % 16
    if e == 0:
        return a
    if e == 8:
        return (-a[0], -a[1])
    if e == 4 or e == 12:
        plus_i = (sign > 0) == (e == 4)
        return (-a[1], a[0]) if plus_i else (a[1], -a[0])
    th = sign * 2.0 * np.pi * e / 16.0
    cr = float(np.cos(th))
    ci = float(np.sin(th))
    return (a[0] * cr - a[1] * ci, a[0] * ci + a[1] * cr)


def _radix16(a, sign):
    b = [None] * 4
    for q in range(4):
        b[q] = _radix4(a[q], a[4 + q], a[8 + q], a[12 + q], sign)
    out = [None] * 16
    for r in range(4):
        c = [_cmul_const(b[q][r], q * r, sign) for q in range(4)]
        y = _radix4(c[0], c[1], c[2], c[3], sign)
        for t in range(4):
            out[r + 4 * t] = y[t]
    return out


def _layernorm0(v):
    m = jnp.mean(v, axis=0, keepdims=True)
    c = v - m
    var = jnp.mean(c * c, axis=0, keepdims=True)
    return c * jax.lax.rsqrt(var + EPS)


def _kernel(x_ref, fdt_ref, wr_ref, wi_ref, mf_hbm, mi_hbm, gdt_hbm, wg_hbm, wu_hbm, wdt_hbm,
            o_ref,
            xs, h_scr, wf, mf_v, mi_v, gdt_v, wg_v, wu_v, wdt_v, wgt, wut, sems):
    step = pl.program_id(0)
    f32 = jnp.float32
    bf16 = jnp.bfloat16

    def _copies():
        pairs = [(mf_hbm, mf_v), (mi_hbm, mi_v), (gdt_hbm, gdt_v),
                 (wg_hbm, wg_v), (wu_hbm, wu_v), (wdt_hbm, wdt_v)]
        return [pltpu.make_async_copy(s, d, sems.at[j]) for j, (s, d) in enumerate(pairs)]

    def _tile_butterflies(sign):
        def body(c, carry):
            r0 = pl.multiple_of(c * 8, 8)
            a = []
            for n in range(NS):
                a.append((xs[pl.ds(r0, 8), n * R:(n + 1) * R],
                          xs[pl.ds(PW + r0, 8), n * R:(n + 1) * R]))
            y = _radix16(a, sign)
            for n in range(NS):
                xs[pl.ds(r0, 8), n * R:(n + 1) * R] = y[n][0]
                xs[pl.ds(PW + r0, 8), n * R:(n + 1) * R] = y[n][1]
            return carry
        jax.lax.fori_loop(0, PW // 8, body, 0)

    @pl.when(step == 0)
    def _spectral():
        cps = _copies()
        for cp in cps:
            cp.start()

        frow = jax.lax.broadcasted_iota(jnp.int32, (R, R), 0)
        for j, w_ref in enumerate((wr_ref, wi_ref)):
            for c in range(NS):
                cols = slice(c * R, (c + 1) * R)
                wf[2 * j, cols, :] = w_ref[:R, cols].astype(f32).T
                hi = jnp.where(frow < DF - R, w_ref[R:, cols].astype(f32), 0.0)
                wf[2 * j + 1, cols, :] = hi.T

        for c in range(S // CN):
            cols = slice(c * CN, (c + 1) * CN)
            xn = _layernorm0(x_ref[:, cols].astype(f32)).astype(bf16)
            xs[:, cols] = jnp.dot(fdt_ref[...], xn, preferred_element_type=f32)

        _tile_butterflies(-1)

        cps[0].wait()
        cps[1].wait()
        for k1 in range(NS):
            cols = slice(k1 * R, (k1 + 1) * R)
            y = xs[:, cols].astype(bf16)
            p = jnp.dot(y, mf_v[pl.ds(k1 * R, R), :], preferred_element_type=f32)
            zr = p[:PW, :R] - p[PW:, R:]
            zi = p[:PW, R:] + p[PW:, :R]
            fr = jnp.concatenate([wf[0, pl.ds(k1, R, stride=NS), :].T,
                                  wf[1, pl.ds(k1, R, stride=NS), :].T], axis=0)
            fi = jnp.concatenate([wf[2, pl.ds(k1, R, stride=NS), :].T,
                                  wf[3, pl.ds(k1, R, stride=NS), :].T], axis=0)
            z = jnp.concatenate([zr * fr - zi * fi, zr * fi + zi * fr], axis=0).astype(bf16)
            q = jnp.dot(z, mi_v[pl.ds(k1 * R, R), :], preferred_element_type=f32)
            xs[:, cols] = jnp.concatenate(
                [q[:PW, :R] - q[PW:, R:], q[:PW, R:] + q[PW:, :R]], axis=0)

        _tile_butterflies(+1)

        cps[2].wait()
        for c in range(S // CN):
            cols = slice(c * CN, (c + 1) * CN)
            y = jnp.dot(gdt_v[...], xs[:, cols].astype(bf16), preferred_element_type=f32)
            h_scr[:, cols] = x_ref[:, cols] + y.astype(bf16)

        cps[3].wait()
        cps[4].wait()
        cps[5].wait()
        for c in range(F // FC):
            wgt[c * FC:(c + 1) * FC, :] = wg_v[:, c * FC:(c + 1) * FC].T
            wut[c * FC:(c + 1) * FC, :] = wu_v[:, c * FC:(c + 1) * FC].T

    cols = pl.ds(pl.multiple_of(step * BN, BN), BN)
    h = h_scr[:, cols]
    ln = _layernorm0(h.astype(f32)).astype(bf16)
    acc = jnp.zeros((D, BN), f32)
    for c in range(F // FC):
        g = jnp.dot(wgt[c * FC:(c + 1) * FC, :], ln, preferred_element_type=f32)
        u = jnp.dot(wut[c * FC:(c + 1) * FC, :], ln, preferred_element_type=f32)
        a = (g * u).astype(bf16)
        acc = acc + jnp.dot(wdt_v[:, c * FC:(c + 1) * FC], a, preferred_element_type=f32)
    o_ref[...] = h + acc.astype(bf16)


@jax.jit
def pallas_sequential_preLN__spectral_gfnet__glu_gated_bilinear__prompt_kernel(
    A_x: jax.Array,
    A_w_r: jax.Array,
    A_w_i: jax.Array,
    B_x: jax.Array,
    B_w_gate: jax.Array,
    B_w_up: jax.Array,
    B_w_down: jax.Array,
):
    del B_x
    xt = A_x.reshape(S, D).T
    fdt, gdt, mf, mi = _dft_constants()
    full = lambda shape: pl.BlockSpec(shape, lambda i: (0,) * len(shape))
    hbm = pl.BlockSpec(memory_space=pl.ANY)
    out = pl.pallas_call(
        _kernel,
        grid=(S // BN,),
        in_specs=[full((D, S)), full((2 * PW, D)), full((PW, S)), full((PW, S)),
                  hbm, hbm, hbm, hbm, hbm, hbm],
        out_specs=pl.BlockSpec((D, BN), lambda i: (0, i)),
        out_shape=jax.ShapeDtypeStruct((D, S), jnp.bfloat16),
        scratch_shapes=[
            pltpu.VMEM((2 * PW, S), jnp.float32),
            pltpu.VMEM((D, S), jnp.bfloat16),
            pltpu.VMEM((4, S, R), jnp.float32),
            pltpu.VMEM((NS * R, 2 * R), jnp.bfloat16),
            pltpu.VMEM((NS * R, 2 * R), jnp.bfloat16),
            pltpu.VMEM((D, 2 * PW), jnp.bfloat16),
            pltpu.VMEM((D, F), jnp.bfloat16),
            pltpu.VMEM((D, F), jnp.bfloat16),
            pltpu.VMEM((D, F), jnp.bfloat16),
            pltpu.VMEM((F, D), jnp.bfloat16),
            pltpu.VMEM((F, D), jnp.bfloat16),
            pltpu.SemaphoreType.DMA((6,)),
        ],
        compiler_params=pltpu.CompilerParams(
            dimension_semantics=("arbitrary",),
            vmem_limit_bytes=100 * 1024 * 1024,
        ),
    )(xt, fdt, A_w_r.T, A_w_i.T,
      mf, mi, gdt, B_w_gate, B_w_up, B_w_down.T)
    return out.T.reshape(1, S, D)
```

```python
import numpy as np
import jax
import jax.numpy as jnp
import jax.experimental.pallas as pl
import jax.experimental.pallas.tpu as pltpu

S = 2048
D = 448
DF = D // 2 + 1
F = 1792
NS = 16
R = 128
PW = 256
EPS = 1e-5
BN = 512
FC = 256
CN = 512


def _dft_constants():
    d = np.arange(D)[None, :]
    f = np.arange(DF)[:, None]
    ang = 2.0 * np.pi * ((d * f) % D) / D
    fdt = np.zeros((2 * PW, D), np.float64)
    fdt[:DF] = np.cos(ang)
    fdt[PW:PW + DF] = -np.sin(ang)
    c = np.full((DF,), 2.0)
    c[0] = 1.0
    c[DF - 1] = 1.0
    gdt = np.zeros((D, 2 * PW), np.float64)
    gdt[:, :DF] = (c[:, None] * np.cos(ang)).T / (D * S)
    gdt[:, PW:PW + DF] = -(c[:, None] * np.sin(ang)).T / (D * S)
    n2 = np.arange(R)
    k2 = np.arange(R)
    mf = np.zeros((NS, R, 2 * R), np.float64)
    mi = np.zeros((NS, R, 2 * R), np.float64)
    for k1 in range(NS):
        a = 2.0 * np.pi * ((n2[:, None] * (k1 + NS * k2)[None, :]) % S) / S
        mf[k1, :, :R] = np.cos(a)
        mf[k1, :, R:] = -np.sin(a)
        mi[k1, :, :R] = np.cos(a.T)
        mi[k1, :, R:] = np.sin(a.T)
    bf = jnp.bfloat16
    return (jnp.asarray(fdt, bf), jnp.asarray(gdt, bf),
            jnp.asarray(mf.reshape(NS * R, 2 * R), bf),
            jnp.asarray(mi.reshape(NS * R, 2 * R), bf))


def _radix4(a0, a1, a2, a3, sign):
    t0 = (a0[0] + a2[0], a0[1] + a2[1])
    t1 = (a0[0] - a2[0], a0[1] - a2[1])
    t2 = (a1[0] + a3[0], a1[1] + a3[1])
    t3 = (a1[0] - a3[0], a1[1] - a3[1])
    y0 = (t0[0] + t2[0], t0[1] + t2[1])
    y2 = (t0[0] - t2[0], t0[1] - t2[1])
    if sign < 0:
        y1 = (t1[0] + t3[1], t1[1] - t3[0])
        y3 = (t1[0] - t3[1], t1[1] + t3[0])
    else:
        y1 = (t1[0] - t3[1], t1[1] + t3[0])
        y3 = (t1[0] + t3[1], t1[1] - t3[0])
    return y0, y1, y2, y3


def _cmul_const(a, e, sign):
    e = e % 16
    if e == 0:
        return a
    if e == 8:
        return (-a[0], -a[1])
    if e == 4 or e == 12:
        plus_i = (sign > 0) == (e == 4)
        return (-a[1], a[0]) if plus_i else (a[1], -a[0])
    th = sign * 2.0 * np.pi * e / 16.0
    cr = float(np.cos(th))
    ci = float(np.sin(th))
    return (a[0] * cr - a[1] * ci, a[0] * ci + a[1] * cr)


def _radix16(a, sign):
    b = [None] * 4
    for q in range(4):
        b[q] = _radix4(a[q], a[4 + q], a[8 + q], a[12 + q], sign)
    out = [None] * 16
    for r in range(4):
        c = [_cmul_const(b[q][r], q * r, sign) for q in range(4)]
        y = _radix4(c[0], c[1], c[2], c[3], sign)
        for t in range(4):
            out[r + 4 * t] = y[t]
    return out


def _layernorm0(v):
    m = jnp.mean(v, axis=0, keepdims=True)
    c = v - m
    var = jnp.mean(c * c, axis=0, keepdims=True)
    return c * jax.lax.rsqrt(var + EPS)


def _kernel(x_hbm, fdt_ref, wr_ref, wi_ref, mf_hbm, mi_hbm, gdt_hbm, wg_hbm, wu_hbm, wdt_hbm,
            o_ref,
            x_ref, xs, h_scr, wf, mf_v, mi_v, gdt_v, wg_v, wu_v, wdt_v,
            wgt, wut, sems):
    step = pl.program_id(0)
    f32 = jnp.float32
    bf16 = jnp.bfloat16

    def _copies():
        pairs = [(x_hbm.at[:, pl.ds(c * CN, CN)], x_ref.at[:, pl.ds(c * CN, CN)])
                 for c in range(S // CN)]
        pairs += [(mf_hbm, mf_v), (mi_hbm, mi_v), (gdt_hbm, gdt_v),
                  (wg_hbm, wg_v), (wu_hbm, wu_v), (wdt_hbm, wdt_v)]
        return [pltpu.make_async_copy(a, b, sems.at[j]) for j, (a, b) in enumerate(pairs)]

    def _tile_butterflies(sign):
        def body(c, carry):
            r0 = pl.multiple_of(c * 8, 8)
            a = []
            for n in range(NS):
                a.append((xs[pl.ds(r0, 8), n * R:(n + 1) * R],
                          xs[pl.ds(PW + r0, 8), n * R:(n + 1) * R]))
            y = _radix16(a, sign)
            for n in range(NS):
                xs[pl.ds(r0, 8), n * R:(n + 1) * R] = y[n][0]
                xs[pl.ds(PW + r0, 8), n * R:(n + 1) * R] = y[n][1]
            return carry
        jax.lax.fori_loop(0, PW // 8, body, 0)

    @pl.when(step == 0)
    def _spectral():
        cps = _copies()
        for cp in cps:
            cp.start()

        for c in range(S // CN):
            cols = slice(c * CN, (c + 1) * CN)
            cps[c].wait()
            xn = _layernorm0(x_ref[:, cols].astype(f32)).astype(bf16)
            xs[:, cols] = jnp.dot(fdt_ref[...], xn, preferred_element_type=f32)

        frow = jax.lax.broadcasted_iota(jnp.int32, (R, R), 0)
        for j, w_ref in enumerate((wr_ref, wi_ref)):
            for c in range(NS):
                cols = slice(c * R, (c + 1) * R)
                wf[2 * j, cols, :] = w_ref[:R, cols].astype(f32).T
                hi = jnp.where(frow < DF - R, w_ref[R:, cols].astype(f32), 0.0)
                wf[2 * j + 1, cols, :] = hi.T

        _tile_butterflies(-1)

        cps[4].wait()
        cps[5].wait()
        for k1 in range(NS):
            cols = slice(k1 * R, (k1 + 1) * R)
            y = xs[:, cols].astype(bf16)
            p = jnp.dot(y, mf_v[pl.ds(k1 * R, R), :], preferred_element_type=f32)
            zr = p[:PW, :R] - p[PW:, R:]
            zi = p[:PW, R:] + p[PW:, :R]
            fr = jnp.concatenate([wf[0, pl.ds(k1, R, stride=NS), :].T,
                                  wf[1, pl.ds(k1, R, stride=NS), :].T], axis=0)
            fi = jnp.concatenate([wf[2, pl.ds(k1, R, stride=NS), :].T,
                                  wf[3, pl.ds(k1, R, stride=NS), :].T], axis=0)
            z = jnp.concatenate([zr * fr - zi * fi, zr * fi + zi * fr], axis=0).astype(bf16)
            q = jnp.dot(z, mi_v[pl.ds(k1 * R, R), :], preferred_element_type=f32)
            xs[:, cols] = jnp.concatenate(
                [q[:PW, :R] - q[PW:, R:], q[:PW, R:] + q[PW:, :R]], axis=0)

        _tile_butterflies(+1)

        cps[6].wait()
        cps[7].wait()
        cps[8].wait()
        nwc = (F // FC + S // CN - 1) // (S // CN)
        for c in range(S // CN):
            cols = slice(c * CN, (c + 1) * CN)
            y = jnp.dot(gdt_v[...], xs[:, cols].astype(bf16), preferred_element_type=f32)
            h_scr[:, cols] = x_ref[:, cols] + y.astype(bf16)
            for wc in range(c * nwc, min((c + 1) * nwc, F // FC)):
                wgt[wc * FC:(wc + 1) * FC, :] = wg_v[:, wc * FC:(wc + 1) * FC].T
                wut[wc * FC:(wc + 1) * FC, :] = wu_v[:, wc * FC:(wc + 1) * FC].T

        cps[9].wait()

    cols = pl.ds(pl.multiple_of(step * BN, BN), BN)
    h = h_scr[:, cols]
    ln = _layernorm0(h.astype(f32)).astype(bf16)
    acc = jnp.zeros((D, BN), f32)
    for c in range(F // FC):
        g = jnp.dot(wgt[c * FC:(c + 1) * FC, :], ln, preferred_element_type=f32)
        u = jnp.dot(wut[c * FC:(c + 1) * FC, :], ln, preferred_element_type=f32)
        a = (g * u).astype(bf16)
        acc = acc + jnp.dot(wdt_v[:, c * FC:(c + 1) * FC], a, preferred_element_type=f32)
    o_ref[...] = h + acc.astype(bf16)


@jax.jit
def pallas_sequential_preLN__spectral_gfnet__glu_gated_bilinear__prompt_kernel(
    A_x: jax.Array,
    A_w_r: jax.Array,
    A_w_i: jax.Array,
    B_x: jax.Array,
    B_w_gate: jax.Array,
    B_w_up: jax.Array,
    B_w_down: jax.Array,
):
    del B_x
    xt = A_x.reshape(S, D).T
    fdt, gdt, mf, mi = _dft_constants()
    full = lambda shape: pl.BlockSpec(shape, lambda i: (0,) * len(shape))
    hbm = pl.BlockSpec(memory_space=pl.ANY)
    out = pl.pallas_call(
        _kernel,
        grid=(S // BN,),
        in_specs=[hbm, full((2 * PW, D)), full((PW, S)), full((PW, S)), hbm, hbm, hbm, hbm, hbm, hbm],
        out_specs=pl.BlockSpec((D, BN), lambda i: (0, i)),
        out_shape=jax.ShapeDtypeStruct((D, S), jnp.bfloat16),
        scratch_shapes=[
            pltpu.VMEM((D, S), jnp.bfloat16),
            pltpu.VMEM((2 * PW, S), jnp.float32),
            pltpu.VMEM((D, S), jnp.bfloat16),
            pltpu.VMEM((4, S, R), jnp.float32),
            pltpu.VMEM((NS * R, 2 * R), jnp.bfloat16),
            pltpu.VMEM((NS * R, 2 * R), jnp.bfloat16),
            pltpu.VMEM((D, 2 * PW), jnp.bfloat16),
            pltpu.VMEM((D, F), jnp.bfloat16),
            pltpu.VMEM((D, F), jnp.bfloat16),
            pltpu.VMEM((D, F), jnp.bfloat16),
            pltpu.VMEM((F, D), jnp.bfloat16),
            pltpu.VMEM((F, D), jnp.bfloat16),
            pltpu.SemaphoreType.DMA((10,)),
        ],
        compiler_params=pltpu.CompilerParams(
            dimension_semantics=("arbitrary",),
            vmem_limit_bytes=100 * 1024 * 1024,
        ),
    )(xt, fdt, A_w_r.T, A_w_i.T,
      mf, mi, gdt, B_w_gate, B_w_up, B_w_down.T)
    return out.T.reshape(1, S, D)
```
